```python
import os as _os
_os.environ.setdefault("JAX_PLATFORMS", "cpu")
import jax
import jax.numpy as jnp

def _softmax(x, axis=-1):
    return jax.nn.softmax(x, axis=axis)
def _gelu(x):
    return jax.nn.gelu(x, approximate=True)
def _silu(x):
    return jax.nn.silu(x)
def _sigmoid(x):
    return jax.nn.sigmoid(x)
def _layernorm(x, axis=-1, eps=1e-5):
    m = jnp.mean(x, axis=axis, keepdims=True)
    v = jnp.var(x, axis=axis, keepdims=True)
    return (x - m) / jnp.sqrt(v + eps)
def _scatter_add(tgt, idx, src, axis=0):
    return tgt.at[idx].add(src)
def _segment_sum(src, seg, n):
    return jax.ops.segment_sum(src, seg, n)
class _Rng:
    def __init__(self, key):
        self._k = key
    def _next(self):
        self._k, sub = jax.random.split(self._k)
        return sub
    def normal(self, shape):
        return jax.random.normal(self._next(), shape, dtype=jnp.bfloat16)
    def randint(self, lo, hi, shape):
        return jax.random.randint(self._next(), shape, lo, hi, dtype=jnp.int32)
    def uniform(self, shape, lo=0.0, hi=1.0):
        return jax.random.uniform(self._next(), shape, jnp.bfloat16, lo, hi)
    def permutation(self, n):
        return jax.random.permutation(self._next(), n)


kernel_name = 'standalone__mha_softmax__near_ridge'

def setup_inputs():
    _rng = _Rng(jax.random.key(int.from_bytes(__import__("os").urandom(4), "little")))
    _w = (lambda a: (lambda t: t.astype(jnp.bfloat16) if jnp.issubdtype(t.dtype, jnp.floating) else t)(jnp.asarray(a)))
    B, H, Sq, Sk, D = 8, 16, 192, 1024, 256
    return {
        "q": _w((lambda *s: _rng.normal(s) * 0.4)(B, H, Sq, D)),
        "k": _w((lambda *s: _rng.normal(s) * 0.4)(B, H, Sk, D)),
        "v": _w((lambda *s: _rng.normal(s) * 0.05)(B, H, Sk, D)),
    }

def reference(q, k, v):
    scale = q.shape[-1] ** -0.5
    scores = jnp.einsum("bhqd,bhkd->bhqk", q, k) * scale
    p = _softmax(scores, axis=-1)
    return jnp.einsum("bhqk,bhkd->bhqd", p, v)
```

```python
import jax
import jax.numpy as jnp
from jax import lax
from jax.experimental import pallas as pl
from jax.experimental.pallas import tpu as pltpu

_G = 8
_LX = 2
_NG = 3
_ROWS = 32
_WROWS = 64


@jax.jit
def pallas_standalone__mha_softmax__near_ridge_kernel(q, k, v):
    B, H, Sq, D = q.shape
    Sk = k.shape[2]
    BH = B * H
    G, NG, rows, wrows = _G, _NG, _ROWS, _WROWS
    hs = BH // G
    L = G + _LX
    cpb = Sk // rows // G
    wpc = Sq // wrows
    nq = Sq // rows
    scale = D ** -0.5

    order = [(g, c, s) for g in range(hs - 1) for c in range(wpc) for s in range(G)]
    tail_w = [[] for _ in range(L)]
    per = -(-len(order) // L)
    pos = 0
    for t in range(L):
        h = BH - L + t
        while pos < len(order) and len(tail_w[t]) < per and order[pos][0] * G + order[pos][2] < h:
            tail_w[t].append(order[pos])
            pos += 1
        if h - 1 >= BH - G:
            tail_w[t] += [(hs - 1, c, h - 1 - (BH - G)) for c in range(wpc)]
    assert pos == len(order)

    def kernel(q_hbm, k_hbm, v_hbm, o_hbm, qb, kb, vb, ob, sq, sk, sv, so):
        def read_list(b):
            g = b // G
            j = b % G
            gs = g % NG
            out = []
            tot = cpb * G
            qat = {int((i + 0.5) * tot / nq): i for i in range(nq)}
            row0 = pl.multiple_of(j * (cpb * rows), cpb * rows)
            src0 = pl.multiple_of(g * Sk + row0, cpb * rows)
            span = (G - 1) * hs * Sk + cpb * rows
            ksrc = k_hbm.at[pl.ds(src0, span)]
            vsrc = v_hbm.at[pl.ds(src0, span)]
            kdst = kb.at[gs, :, pl.ds(row0, cpb * rows)]
            vdst = vb.at[gs, :, pl.ds(row0, cpb * rows)]
            qsrc = q_hbm.at[pl.ds(pl.multiple_of((g + j * hs) * Sq, rows), Sq)]
            qdst = qb.at[gs, j]
            n = 0
            for c in range(cpb):
                for s in range(G):
                    for jj, (src, dst, sem) in enumerate(((ksrc, kdst, sk), (vsrc, vdst, sv))):
                        def f(c=c, s=s, jj=jj, src=src, dst=dst, sem=sem):
                            pltpu.make_async_copy(
                                src.at[pl.ds(s * hs * Sk + c * rows, rows)],
                                dst.at[s, pl.ds(c * rows, rows)],
                                sem.at[gs, s]).start(priority=(s + jj) % 2)
                        out.append((jj, f))
                    if n in qat:
                        def f(c=qat[n]):
                            pltpu.make_async_copy(
                                qsrc.at[pl.ds(c * rows, rows)],
                                qdst.at[pl.ds(c * rows, rows)],
                                sq.at[gs, j]).start(priority=c % 2)
                        out.append((2, f))
                    n += 1
            return out

        def write(g, c, s, prio):
            r = (g + s * hs) * Sq + c * wrows
            pltpu.make_async_copy(ob.at[pl.ds(r, wrows)], o_hbm.at[pl.ds(r, wrows)], so.at[0]).start(priority=prio)

        def wait(h):
            g = h // G
            s = h % G
            gs = g % NG
            pltpu.make_async_copy(qb.at[gs, s], qb.at[gs, s], sq.at[gs, s]).wait()
            pltpu.make_async_copy(kb.at[gs, s], kb.at[gs, s], sk.at[gs, s]).wait()
            pltpu.make_async_copy(vb.at[gs, s], vb.at[gs, s], sv.at[gs, s]).wait()

        def compute(h, issue):
            g = h // G
            s_ = h % G
            gs = g % NG
            r = pl.multiple_of((g + s_ * hs) * Sq, rows)
            for kind, f in issue:
                if kind == 1:
                    f()
            s = lax.dot_general(qb[gs, s_], kb[gs, s_], (((1,), (1,)), ((), ())),
                                preferred_element_type=jnp.float32)
            for kind, f in issue:
                if kind != 1:
                    f()
            s = s * scale
            m = jnp.max(s, axis=-1, keepdims=True)
            p = jnp.exp(s - m)
            l = jnp.sum(p, axis=-1, keepdims=True)
            o = jnp.dot(p.astype(vb.dtype), vb[gs, s_], preferred_element_type=jnp.float32)
            ob[pl.ds(r, Sq), :] = (o / l).astype(ob.dtype)

        def prologue(b, _):
            for kind, f in read_list(b):
                f()
        lax.fori_loop(0, L, prologue, None)

        def body(h, _):
            wait(h)
            compute(h, read_list(h + L))
        lax.fori_loop(0, BH - L, body, None)

        def tail(h, _):
            for t in range(L):
                @pl.when(h == BH - L + t)
                def _():
                    for n, (g, c, s) in enumerate(tail_w[t]):
                        write(g, c, s, n % 2)
            wait(h)
            compute(h, [])
        lax.fori_loop(BH - L, BH, tail, None)
        for c in range(wpc):
            write(hs - 1, c, G - 1, c % 2)
        pltpu.make_async_copy(ob, o_hbm, so.at[0]).wait()

    out = pl.pallas_call(
        kernel,
        in_specs=[pl.BlockSpec(memory_space=pl.ANY)] * 3,
        out_specs=pl.BlockSpec(memory_space=pl.ANY),
        out_shape=jax.ShapeDtypeStruct((BH * Sq, D), q.dtype),
        scratch_shapes=[
            pltpu.VMEM((NG, G, Sq, D), q.dtype),
            pltpu.VMEM((NG, G, Sk, D), k.dtype),
            pltpu.VMEM((NG, G, Sk, D), v.dtype),
            pltpu.VMEM((BH * Sq, D), q.dtype),
            pltpu.SemaphoreType.DMA((NG, G)),
            pltpu.SemaphoreType.DMA((NG, G)),
            pltpu.SemaphoreType.DMA((NG, G)),
            pltpu.SemaphoreType.DMA((1,)),
        ],
        compiler_params=pltpu.CompilerParams(
            vmem_limit_bytes=100 * 1024 * 1024, disable_bounds_checks=True),
    )(q.reshape(BH * Sq, D), k.reshape(BH * Sk, D), v.reshape(BH * Sk, D))
    return out.reshape(q.shape)
```

```python
import math

import jax
import jax.numpy as jnp
from jax import lax
from jax.experimental import pallas as pl
from jax.experimental.pallas import tpu as pltpu

_GROUP = 8
_SLOTS = 3
_LOOKAHEAD = 2
_READ_ROWS = 32
_WRITE_ROWS = 64
_WRITE_GROUPS = 2


@jax.jit
def pallas_standalone__mha_softmax__near_ridge_kernel(
    q: jax.Array,
    k: jax.Array,
    v: jax.Array,
):
    B, H, Sq, D = q.shape
    Sk = k.shape[2]
    n_heads = B * H

    n_groups = n_heads // _GROUP
    batch_rows = Sk // _GROUP
    ahead = _GROUP + _LOOKAHEAD
    last_group_step = n_heads - _GROUP
    assert n_heads % _GROUP == 0 and n_groups >= _SLOTS
    assert Sk % (_GROUP * _READ_ROWS) == 0
    assert Sq % _READ_ROWS == 0 and Sq % _WRITE_ROWS == 0
    assert 1 <= _LOOKAHEAD < _GROUP
    write_groups = max(_WRITE_GROUPS, pl.cdiv(n_groups - 1, _GROUP + 1))

    exp2_scale = float(D) ** -0.5 * math.log2(math.e)

    def kernel(q_hbm, k_hbm, v_hbm, o_hbm,
               q_buf, k_buf, v_buf, o_buf, q_sem, k_sem, v_sem, o_sem):

        def position(h):
            g = lax.div(h, _GROUP)
            return g, lax.rem(h, _GROUP), lax.rem(g, _SLOTS)

        def start_reads(h):
            g, j, slot = position(h)
            row = pl.multiple_of(j * batch_rows, batch_rows)
            src_row = pl.multiple_of(g * Sk + row, batch_rows)
            span = (_GROUP - 1) * n_groups * Sk + batch_rows
            kv = (
                (k_hbm.at[pl.ds(src_row, span)],
                 k_buf.at[slot, :, pl.ds(row, batch_rows)], k_sem.at[slot]),
                (v_hbm.at[pl.ds(src_row, span)],
                 v_buf.at[slot, :, pl.ds(row, batch_rows)], v_sem.at[slot]),
            )
            q_row = pl.multiple_of((g + j * n_groups) * Sq, _READ_ROWS)
            q_src, q_dst = q_hbm.at[pl.ds(q_row, Sq)], q_buf.at[slot, j]

            pieces = [(c, s) for c in range(0, batch_rows, _READ_ROWS)
                      for s in range(_GROUP)]
            n_q = Sq // _READ_ROWS
            q_started = 0
            for n, (c, s) in enumerate(pieces):
                for thread, (src, dst, sem) in enumerate(kv):
                    pltpu.make_async_copy(
                        src.at[pl.ds(s * n_groups * Sk + c, _READ_ROWS)],
                        dst.at[s, pl.ds(c, _READ_ROWS)],
                        sem,
                    ).start(priority=thread)
                while q_started < n_q and (
                        (2 * q_started + 1) * len(pieces) < 2 * n_q * (n + 1)):
                    rows = pl.ds(q_started * _READ_ROWS, _READ_ROWS)
                    pltpu.make_async_copy(
                        q_src.at[rows], q_dst.at[rows], q_sem.at[slot],
                    ).start(priority=q_started % 2)
                    q_started += 1
            assert q_started == n_q

        def wait_group(buf, sem, h):
            slot = position(h)[2]
            pltpu.make_async_copy(buf.at[slot], buf.at[slot], sem.at[slot]).wait()

        def attend(h):
            g, j, slot = position(h)
            s = lax.dot_general(
                q_buf[slot, j], k_buf[slot, j], (((1,), (1,)), ((), ())),
                preferred_element_type=jnp.float32)
            m = jnp.max(s, axis=-1, keepdims=True)
            p = jnp.exp2((s - m) * exp2_scale)
            l = jnp.sum(p, axis=-1, keepdims=True)
            o = jnp.dot(p.astype(v_buf.dtype), v_buf[slot, j],
                        preferred_element_type=jnp.float32)
            row = pl.multiple_of((g + j * n_groups) * Sq, _WRITE_ROWS)
            o_buf[pl.ds(row, Sq), :] = (o / l).astype(o_buf.dtype)

        def start_group_write(g, _):
            row = pl.multiple_of(g * Sq, _WRITE_ROWS)
            span = pl.ds(row, (_GROUP - 1) * n_groups * Sq + Sq)
            src, dst = o_buf.at[span], o_hbm.at[span]
            pieces = [(c, s) for c in range(0, Sq, _WRITE_ROWS)
                      for s in range(_GROUP)]
            for n, (c, s) in enumerate(pieces):
                rows = pl.ds(s * n_groups * Sq + c, _WRITE_ROWS)
                pltpu.make_async_copy(
                    src.at[rows], dst.at[rows], o_sem.at[0],
                ).start(priority=n % 2)

        def start_head_write(h):
            g, j, _ = position(h)
            row = pl.multiple_of((g + j * n_groups) * Sq, _WRITE_ROWS)
            src, dst = o_buf.at[pl.ds(row, Sq)], o_hbm.at[pl.ds(row, Sq)]
            for n, c in enumerate(range(0, Sq, _WRITE_ROWS)):
                rows = pl.ds(c, _WRITE_ROWS)
                pltpu.make_async_copy(
                    src.at[rows], dst.at[rows], o_sem.at[0],
                ).start(priority=n % 2)

        lax.fori_loop(0, ahead, lambda h, _: start_reads(h), None)

        def read_phase(h, _):
            @pl.when(lax.rem(h, _GROUP) == 0)
            def _():
                wait_group(q_buf, q_sem, h)
                wait_group(k_buf, k_sem, h)
                wait_group(v_buf, v_sem, h)

            attend(h)
            start_reads(h + ahead)

        lax.fori_loop(0, n_heads - ahead, read_phase, None)

        def write_phase(h, _):
            @pl.when(h == last_group_step - 1)
            def _():
                wait_group(k_buf, k_sem, last_group_step)

            @pl.when(h >= last_group_step - 1)
            def _():
                t = h - (last_group_step - 1)
                lax.fori_loop(
                    jnp.minimum(t * write_groups, lax.div(h - 1, _GROUP)),
                    jnp.minimum((t + 1) * write_groups, lax.div(h, _GROUP)),
                    start_group_write, None)

            @pl.when(h == last_group_step)
            def _():
                wait_group(q_buf, q_sem, h)
                wait_group(v_buf, v_sem, h)

            attend(h)

            @pl.when(h >= last_group_step)
            def _():
                start_head_write(h)

        lax.fori_loop(n_heads - ahead, n_heads, write_phase, None)
        pltpu.make_async_copy(o_buf, o_hbm, o_sem.at[0]).wait()

    out = pl.pallas_call(
        kernel,
        in_specs=[pl.BlockSpec(memory_space=pl.ANY)] * 3,
        out_specs=pl.BlockSpec(memory_space=pl.ANY),
        out_shape=jax.ShapeDtypeStruct((n_heads * Sq, D), q.dtype),
        scratch_shapes=[
            pltpu.VMEM((_SLOTS, _GROUP, Sq, D), q.dtype),
            pltpu.VMEM((_SLOTS, _GROUP, Sk, D), k.dtype),
            pltpu.VMEM((_SLOTS, _GROUP, Sk, D), v.dtype),
            pltpu.VMEM((n_heads * Sq, D), q.dtype),
            pltpu.SemaphoreType.DMA((_SLOTS,)),
            pltpu.SemaphoreType.DMA((_SLOTS,)),
            pltpu.SemaphoreType.DMA((_SLOTS,)),
            pltpu.SemaphoreType.DMA((1,)),
        ],
        compiler_params=pltpu.CompilerParams(
            vmem_limit_bytes=64 * 1024 * 1024,
            disable_bounds_checks=True,
            disable_semaphore_checks=True,
        ),
    )(q.reshape(n_heads * Sq, D),
      k.reshape(n_heads * Sk, D),
      v.reshape(n_heads * Sk, D))
    return out.reshape(B, H, Sq, D)
```

```python
import math

import jax
import jax.numpy as jnp
from jax import lax
from jax.experimental import pallas as pl
from jax.experimental.pallas import tpu as pltpu

_GROUP = 8
_SLOTS = 3
_LOOKAHEAD = 3
_READ_ROWS = 32
_READ_HEADS = 2
_WRITE_ROWS = 64
_WRITE_GROUPS = 2


@jax.jit
def pallas_standalone__mha_softmax__near_ridge_kernel(
    q: jax.Array,
    k: jax.Array,
    v: jax.Array,
):
    B, H, Sq, D = q.shape
    Sk = k.shape[2]
    n_heads = B * H

    n_groups = n_heads // _GROUP
    batch_rows = Sk // _GROUP
    ahead = _GROUP + _LOOKAHEAD
    last_group_step = n_heads - _GROUP
    write_groups = max(_WRITE_GROUPS, pl.cdiv(n_groups - 1, _GROUP + 1))
    assert n_heads % _GROUP == 0 and n_groups >= _SLOTS
    assert _GROUP % _READ_HEADS == 0 and 1 <= _LOOKAHEAD < _GROUP
    assert Sk % (_GROUP * _READ_ROWS) == 0
    assert Sq % _READ_ROWS == 0 and Sq % _WRITE_ROWS == 0

    exp2_scale = float(D) ** -0.5 * math.log2(math.e)

    def kernel(q_hbm, k_hbm, v_hbm, o_hbm,
               q_buf, k_buf, v_buf, o_buf, q_sem, k_sem, v_sem, o_sem):

        def position(h):
            g = lax.div(h, _GROUP)
            return g, lax.rem(h, _GROUP), lax.rem(g, _SLOTS)

        def start_reads(h):
            g, j, slot = position(h)
            batch = pl.ds(pl.multiple_of(j * batch_rows, batch_rows), batch_rows)
            kv = (
                (k_hbm.at[:, g, batch], k_buf.at[slot, :, batch], k_sem.at[slot]),
                (v_hbm.at[:, g, batch], v_buf.at[slot, :, batch], v_sem.at[slot]),
            )
            q_src, q_dst = q_hbm.at[j, g], q_buf.at[slot, j]

            pieces = [(pl.ds(-s % _GROUP, _READ_HEADS), pl.ds(c, _READ_ROWS))
                      for c in range(0, batch_rows, _READ_ROWS)
                      for s in range(0, _GROUP, _READ_HEADS)]
            n_q, q_started = Sq // _READ_ROWS, 0
            for n, piece in enumerate(pieces):
                for thread, (src, dst, sem) in enumerate(kv):
                    pltpu.make_async_copy(
                        src.at[piece], dst.at[piece], sem,
                    ).start(priority=thread)
                while q_started < n_q and (
                        (2 * q_started + 1) * len(pieces) < 2 * n_q * (n + 1)):
                    rows = pl.ds(q_started * _READ_ROWS, _READ_ROWS)
                    pltpu.make_async_copy(
                        q_src.at[rows], q_dst.at[rows], q_sem.at[slot],
                    ).start(priority=q_started % 2)
                    q_started += 1
            assert q_started == n_q

        def wait_group(buf, sem, h):
            slot = position(h)[2]
            pltpu.make_async_copy(buf.at[slot], buf.at[slot], sem.at[slot]).wait()

        def attend(h):
            g, j, slot = position(h)
            s = lax.dot_general(
                q_buf[slot, j], k_buf[slot, j], (((1,), (1,)), ((), ())),
                preferred_element_type=jnp.float32)
            m = jnp.max(s, axis=-1, keepdims=True)
            p = jnp.exp2((s - m) * exp2_scale)
            l = jnp.sum(p, axis=-1, keepdims=True)
            o = jnp.dot(p.astype(v_buf.dtype), v_buf[slot, j],
                        preferred_element_type=jnp.float32)
            o_buf[j, g] = (o / l).astype(o_buf.dtype)

        def start_group_write(g, _):
            src, dst = o_buf.at[:, g], o_hbm.at[:, g]
            pieces = [(s, pl.ds(c, _WRITE_ROWS))
                      for c in range(0, Sq, _WRITE_ROWS) for s in range(_GROUP)]
            for n, piece in enumerate(pieces):
                pltpu.make_async_copy(
                    src.at[piece], dst.at[piece], o_sem.at[0],
                ).start(priority=n % 2)

        def start_head_write(h):
            g, j, _ = position(h)
            src, dst = o_buf.at[j, g], o_hbm.at[j, g]
            for n, c in enumerate(range(0, Sq, _WRITE_ROWS)):
                rows = pl.ds(c, _WRITE_ROWS)
                pltpu.make_async_copy(
                    src.at[rows], dst.at[rows], o_sem.at[0],
                ).start(priority=n % 2)

        lax.fori_loop(0, ahead, lambda h, _: start_reads(h), None)

        def read_phase(h, _):
            @pl.when(lax.rem(h, _GROUP) == 0)
            def _():
                wait_group(q_buf, q_sem, h)
                wait_group(k_buf, k_sem, h)
                wait_group(v_buf, v_sem, h)

            attend(h)
            start_reads(h + ahead)

        lax.fori_loop(0, n_heads - ahead, read_phase, None)

        def write_phase(h, _):
            @pl.when(h == last_group_step - 1)
            def _():
                wait_group(k_buf, k_sem, last_group_step)

            @pl.when(h >= last_group_step - 1)
            def _():
                t = h - (last_group_step - 1)
                lax.fori_loop(
                    jnp.minimum(t * write_groups, lax.div(h - 1, _GROUP)),
                    jnp.minimum((t + 1) * write_groups, lax.div(h, _GROUP)),
                    start_group_write, None)

            @pl.when(h == last_group_step)
            def _():
                wait_group(q_buf, q_sem, h)
                wait_group(v_buf, v_sem, h)

            attend(h)

            @pl.when(h >= last_group_step)
            def _():
                start_head_write(h)

        lax.fori_loop(n_heads - ahead, n_heads, write_phase, None)
        pltpu.make_async_copy(o_buf, o_hbm, o_sem.at[0]).wait()

    out = pl.pallas_call(
        kernel,
        in_specs=[pl.BlockSpec(memory_space=pl.ANY)] * 3,
        out_specs=pl.BlockSpec(memory_space=pl.ANY),
        out_shape=jax.ShapeDtypeStruct((_GROUP, n_groups, Sq, D), q.dtype),
        scratch_shapes=[
            pltpu.VMEM((_SLOTS, _GROUP, Sq, D), q.dtype),
            pltpu.VMEM((_SLOTS, _GROUP, Sk, D), k.dtype),
            pltpu.VMEM((_SLOTS, _GROUP, Sk, D), v.dtype),
            pltpu.VMEM((_GROUP, n_groups, Sq, D), q.dtype),
            pltpu.SemaphoreType.DMA((_SLOTS,)),
            pltpu.SemaphoreType.DMA((_SLOTS,)),
            pltpu.SemaphoreType.DMA((_SLOTS,)),
            pltpu.SemaphoreType.DMA((1,)),
        ],
        compiler_params=pltpu.CompilerParams(
            vmem_limit_bytes=64 * 1024 * 1024,
            disable_bounds_checks=True,
            disable_semaphore_checks=True,
        ),
    )(q.reshape(_GROUP, n_groups, Sq, D),
      k.reshape(_GROUP, n_groups, Sk, D),
      v.reshape(_GROUP, n_groups, Sk, D))
    return out.reshape(B, H, Sq, D)
```
